```python
import jax
import jax.numpy as jnp

def _softmax(x, axis=-1):
    return jax.nn.softmax(x, axis=axis)
def _gelu(x):
    return jax.nn.gelu(x, approximate=True)
def _silu(x):
    return jax.nn.silu(x)
def _sigmoid(x):
    return jax.nn.sigmoid(x)
def _layernorm(x, axis=-1, eps=1e-5):
    m = jnp.mean(x, axis=axis, keepdims=True)
    v = jnp.var(x, axis=axis, keepdims=True)
    return (x - m) / jnp.sqrt(v + eps)
def _scatter_add(tgt, idx, src, axis=0):
    return tgt.at[idx].add(src)
def _segment_sum(src, seg, n):
    return jax.ops.segment_sum(src, seg, n)
class _Rng:
    def __init__(self, key):
        self._k = key
    def _next(self):
        self._k, sub = jax.random.split(self._k)
        return sub
    def normal(self, shape):
        return jax.random.normal(self._next(), shape, dtype=jnp.bfloat16)
    def randint(self, lo, hi, shape):
        return jax.random.randint(self._next(), shape, lo, hi, dtype=jnp.int32)
    def uniform(self, shape, lo=0.0, hi=1.0):
        return jax.random.uniform(self._next(), shape, jnp.bfloat16, lo, hi)
    def permutation(self, n):
        return jax.random.permutation(self._next(), n)


kernel_name = 'standalone__instancenorm__prompt'

def setup_inputs():
    _rng = _Rng(jax.random.key(int.from_bytes(__import__("os").urandom(4), "little")))
    _w = (lambda a: (lambda t: t.astype(jnp.bfloat16) if jnp.issubdtype(t.dtype, jnp.floating) else t)(jnp.asarray(a)))
    B, C, H, W = 2, 1024, 2048, 32
    return {
        "x": _w((lambda *s: _rng.normal(s) * 0.05)(B, C, H, W)),
        "g": _w((lambda *s: _rng.normal(s) * 0.05)(C) + 1.0),
        "b": _w((lambda *s: _rng.normal(s) * 0.05)(C)),
    }

def reference(x, g, b):
    mu = x.mean(axis=(-2, -1), keepdims=True)
    var = ((x - mu) * (x - mu)).mean(axis=(-2, -1), keepdims=True)
    xhat = (x - mu) / jnp.sqrt(var + 1e-5)
    return xhat * g.reshape(1, -1, 1, 1) + b.reshape(1, -1, 1, 1)
```

```python
import jax
import jax.numpy as jnp
from jax import lax
import jax.experimental.pallas as pl
import jax.experimental.pallas.tpu as pltpu

_EPS = 1e-5
_LANES = 128
_ROWS = 8

_NS = 16
_Q = 8
_CHUNK = 6

_R_STREAMS, _R_COLS = 2, 1024
_R_ORDER = (0, 4, 1, 5, 2, 6, 3, 7)
_R_LAG = 2
_R_TAIL = 3

_W_STREAMS, _W_COLS = 4, 1024
_W_LAG = 4
_W_TAIL = 1
_AHEAD = 2

_C_ROWS, _C_COLS = 16, 256


def _div(i, n):
    assert n & (n - 1) == 0
    return lax.shift_right_logical(i, n.bit_length() - 1)


def _mod(i, n):
    assert n & (n - 1) == 0
    return i & (n - 1)


def _loop(lo, hi, body):
    def wrapped(i, carry):
        body(i)
        return carry

    lax.fori_loop(lo, hi, wrapped, 0)


def _make_kernel(B, C, H, W):
    nblk = B * C // (_NS * _Q)
    nchunks = pl.cdiv(nblk, _CHUNK)
    r_cb = H // _R_COLS
    r_rounds = (W // _ROWS) * r_cb
    groups = _NS // _W_STREAMS
    w_rounds = W // _ROWS
    inv_n = 1.0 / (H * W)
    tiles = [
        (pl.ds(h * _C_ROWS, _C_ROWS), pl.ds(cb * _C_COLS, _C_COLS))
        for h in range(W // _C_ROWS)
        for cb in range(H // _C_COLS)
    ]

    def kernel(x_hbm, g_hbm, b_hbm, o_hbm, buf, gb, gt, bt, r_sem, w_sem, gb_sem):
        def r_piece(u, p):
            rr = pl.ds((p // r_cb) * _ROWS, _ROWS)
            cc = pl.ds((p % r_cb) * _R_COLS, _R_COLS)
            sem = r_sem.at[_mod(u, _R_LAG) * r_rounds + p]
            return _div(u, _Q), _mod(u, _Q), rr, cc, sem

        def r_start(b0, u, p):
            k, j, rr, cc, sem = r_piece(u, p)
            for i, s in enumerate(_R_ORDER):
                ss = pl.ds(s * _R_STREAMS, _R_STREAMS)
                pltpu.make_async_copy(
                    x_hbm.at[b0 + k, ss, j, rr, cc], buf.at[k, ss, j, rr, cc], sem
                ).start(priority=i % 2)

        def r_wait(u, p):
            k, j, rr, cc, sem = r_piece(u, p)
            dst = buf.at[k, :, j, rr, cc]
            pltpu.make_async_copy(dst, dst, sem).wait()

        def r_column(b0, u):
            for p in range(r_rounds):
                r_start(b0, u, p)

        def unit(v):
            k = _div(v, groups * _Q)
            return k, _mod(_div(v, _Q), groups) * _W_STREAMS, _mod(v, _Q)

        def w_start(b0, v, p):
            k, s0, j = unit(v)
            for cb in range(H // _W_COLS):
                idx = (
                    pl.ds(s0, _W_STREAMS),
                    j,
                    pl.ds(p * _ROWS, _ROWS),
                    pl.ds(cb * _W_COLS, _W_COLS),
                )
                pltpu.make_async_copy(
                    buf.at[(k,) + idx],
                    o_hbm.at[(b0 + k,) + idx],
                    w_sem.at[_mod(v, _W_LAG) * w_rounds + p],
                ).start()

        def w_wait(v, p):
            k, s0, j = unit(v)
            src = buf.at[k, pl.ds(s0, _W_STREAMS), j, pl.ds(p * _ROWS, _ROWS)]
            sem = w_sem.at[_mod(v, _W_LAG) * w_rounds + p]
            pltpu.make_async_copy(src, src, sem).wait()

        def total(acc):
            return jnp.sum(jnp.sum(acc, axis=1, keepdims=True), axis=0, keepdims=True)

        def normalise(b0, v):
            k, s0, j = unit(v)
            means = []
            for s in range(_W_STREAMS):
                acc = None
                for rr, cc in tiles:
                    val = buf[k, s0 + s, j, rr, cc].astype(jnp.float32)
                    acc = val if acc is None else acc + val
                means.append(total(acc) * inv_n)
            affine = []
            for s in range(_W_STREAMS):
                acc = None
                for rr, cc in tiles:
                    val = buf[k, s0 + s, j, rr, cc].astype(jnp.float32) - means[s]
                    val = val * val
                    acc = val if acc is None else acc + val
                ch = _mod(((b0 + k) * _NS + s0 + s) * _Q + j, C)
                scale = lax.rsqrt(total(acc) * inv_n + _EPS) * gt[pl.ds(ch, 1), :]
                shift = bt[pl.ds(ch, 1), :] - means[s] * scale
                reps = _C_COLS // _LANES
                affine.append(
                    (
                        jnp.concatenate([scale] * reps, axis=1),
                        jnp.concatenate([shift] * reps, axis=1),
                    )
                )
            for s in range(_W_STREAMS):
                scale, shift = affine[s]
                for rr, cc in tiles:
                    val = buf[k, s0 + s, j, rr, cc].astype(jnp.float32)
                    buf[k, s0 + s, j, rr, cc] = (val * scale + shift).astype(buf.dtype)

        r_column(0, jnp.int32(0))
        gb_copies = [
            pltpu.make_async_copy(src, gb.at[i], gb_sem.at[i])
            for i, src in enumerate((g_hbm, b_hbm))
        ]
        for copy in gb_copies:
            copy.start()

        def chunk(c):
            b0 = c * _CHUNK
            nb = jnp.minimum(nblk - b0, _CHUNK)
            ncol, nunit = nb * _Q, nb * (groups * _Q)

            def read(u):
                for p in range(r_rounds):
                    r_wait(u - _R_LAG, p)
                    r_start(b0, u, p)

            _loop(1, _R_LAG, lambda u: r_column(b0, u))
            _loop(_R_LAG, ncol, read)

            def r_drain(lo, hi):
                for t in range(lo, hi):
                    r_wait(ncol - _R_LAG + t // r_rounds, t % r_rounds)

            @pl.when(c == 0)
            def _():
                for i, dst in enumerate((gt, bt)):
                    gb_copies[i].wait()
                    val = gb[i].astype(jnp.float32)
                    for t in range(C // _LANES):
                        dst[pl.ds(t * _LANES, _LANES), :] = jnp.broadcast_to(
                            val[t : t + 1, :], (_LANES, _LANES)
                        ).T

            def write(v):
                @pl.when(v == 0)
                def _():
                    r_drain(0, _R_LAG * r_rounds - _R_TAIL)

                @pl.when(v >= _W_LAG)
                def _():
                    for p in range(w_rounds):
                        w_wait(v - _W_LAG, p)

                @pl.when(v >= 0)
                def _():
                    for p in range(w_rounds):
                        w_start(b0, v, p)

                @pl.when(v == _AHEAD)
                def _():
                    r_drain(_R_LAG * r_rounds - _R_TAIL, _R_LAG * r_rounds)

                @pl.when(v + _AHEAD < nunit)
                def _():
                    normalise(b0, v + _AHEAD)

            _loop(-_AHEAD, nunit, write)

            def w_drain(lo, hi):
                for t in range(lo, hi):
                    w_wait(nunit - _W_LAG + t // w_rounds, t % w_rounds)

            w_drain(0, _W_LAG * w_rounds - _W_TAIL)

            @pl.when(c + 1 < nchunks)
            def _():
                r_column(b0 + nb, jnp.int32(0))

            w_drain(_W_LAG * w_rounds - _W_TAIL, _W_LAG * w_rounds)

        _loop(0, nchunks, chunk)

    scratch = [
        pltpu.VMEM((_CHUNK, _NS, _Q, W, H), jnp.bfloat16),
        pltpu.VMEM((2, C // _LANES, _LANES), jnp.bfloat16),
        pltpu.VMEM((C, _LANES), jnp.float32),
        pltpu.VMEM((C, _LANES), jnp.float32),
        pltpu.SemaphoreType.DMA((_R_LAG * r_rounds,)),
        pltpu.SemaphoreType.DMA((_W_LAG * w_rounds,)),
        pltpu.SemaphoreType.DMA((2,)),
    ]
    return kernel, scratch


@jax.jit
def pallas_standalone__instancenorm__prompt_kernel(
    x: jax.Array,
    g: jax.Array,
    b: jax.Array,
):
    B, C, H, W = x.shape
    kernel, scratch = _make_kernel(B, C, H, W)
    xt = jnp.transpose(x, (0, 1, 3, 2)).reshape(B * C // (_NS * _Q), _NS, _Q, W, H)
    y = pl.pallas_call(
        kernel,
        in_specs=[pl.BlockSpec(memory_space=pl.ANY)] * 3,
        out_specs=pl.BlockSpec(memory_space=pl.ANY),
        out_shape=jax.ShapeDtypeStruct(xt.shape, xt.dtype),
        scratch_shapes=scratch,
        compiler_params=pltpu.CompilerParams(
            vmem_limit_bytes=110 * 1024 * 1024, disable_bounds_checks=True
        ),
    )(xt, g.reshape(C // _LANES, _LANES), b.reshape(C // _LANES, _LANES))
    return jnp.transpose(y.reshape(B, C, W, H), (0, 1, 3, 2))
```

```python
import jax
import jax.numpy as jnp
from jax import lax
import jax.experimental.pallas as pl
import jax.experimental.pallas.tpu as pltpu

_EPS = 1e-5
_LANES = 128

_Q = 8
_CHUNK = 96
_P_ROWS, _P_COLS = 8, 1024

_R_STRIPES, _R_PAIR = 16, 2
_R_ORDER = (0, 4, 1, 5, 2, 6, 3, 7)
_R_LAG = 4
_R_TAIL = 3

_W_NARROW, _W_WIDE = 6, 8
_W_LAG = 2
_W_TAIL = 1
_AHEAD = 2

_C_ROWS, _C_COLS = 16, 256


def _div(i, n):
    assert n & (n - 1) == 0
    return lax.shift_right_logical(i, n.bit_length() - 1)


def _mod(i, n):
    assert n & (n - 1) == 0
    return i & (n - 1)


def _loop(lo, hi, body):
    def wrapped(i, carry):
        body(i)
        return carry

    lax.fori_loop(lo, hi, wrapped, 0)


def _plan(stripes):
    plan = []
    for first in range(0, stripes, _CHUNK):
        size = min(_CHUNK, stripes - first)
        assert size % _R_STRIPES == 0
        wide = next(
            n for n in range(_W_NARROW) if (size - n * _W_WIDE) % _W_NARROW == 0
        )
        narrow = (size - wide * _W_WIDE) // _W_NARROW
        plan.append((first, size // _R_STRIPES * _Q, narrow * _Q, (narrow + wide) * _Q))
    return plan


def _make_kernel(B, C, H, W):
    plan = _plan(B * C // _Q)
    pieces = [
        (pl.ds(r, _P_ROWS), pl.ds(c, _P_COLS))
        for r in range(0, W, _P_ROWS)
        for c in range(0, H, _P_COLS)
    ]
    tiles = [
        (pl.ds(r, _C_ROWS), pl.ds(c, _C_COLS))
        for r in range(0, W, _C_ROWS)
        for c in range(0, H, _C_COLS)
    ]
    n_pieces = len(pieces)
    inv_n = 1.0 / (H * W)

    def lookup(c):
        out = [jnp.int32(a) for a in plan[0]]
        for i in range(1, len(plan)):
            out = [jnp.where(c == i, a, o) for a, o in zip(plan[i], out)]
        return out

    def group_start(narrow, v):
        wide_before = _div(jnp.maximum(v - narrow, 0), _Q)
        return _div(v, _Q) * _W_NARROW + wide_before * (_W_WIDE - _W_NARROW)

    def by_width(narrow, v, body):
        pl.when(v < narrow)(lambda: body(_W_NARROW))
        pl.when(v >= narrow)(lambda: body(_W_WIDE))

    def total(acc):
        return jnp.sum(jnp.sum(acc, axis=1, keepdims=True), axis=0, keepdims=True)

    def kernel(x_hbm, g_hbm, b_hbm, o_hbm, buf, gb, gt, bt, r_sem, w_sem, gb_sem):
        def r_copies(first, columns, u, lo, hi):
            s0, j = _div(u, _Q) * _R_STRIPES, _mod(u, _Q)
            copies = []
            for p in range(lo, hi):
                slot = _mod(u, _R_LAG)
                if p >= n_pieces - _R_TAIL:
                    slot = jnp.where(u == columns - 1, _R_LAG, slot)
                for pair in _R_ORDER:
                    s = s0 + pair * _R_PAIR
                    copies.append(
                        pltpu.make_async_copy(
                            x_hbm.at[(pl.ds(first + s, _R_PAIR), j) + pieces[p]],
                            buf.at[(pl.ds(s, _R_PAIR), j) + pieces[p]],
                            r_sem.at[slot],
                        )
                    )
            return copies

        def r_wait_column(u):
            dst = buf.at[pl.ds(_div(u, _Q) * _R_STRIPES, _R_STRIPES), _mod(u, _Q)]
            pltpu.make_async_copy(dst, dst, r_sem.at[_mod(u, _R_LAG)]).wait()

        def w_copies(first, narrow, units, v, width, lo, hi):
            s, j = group_start(narrow, v), _mod(v, _Q)
            copies = []
            for p in range(lo, hi):
                slot = _mod(v, _W_LAG)
                if p >= n_pieces - _W_TAIL:
                    slot = jnp.where(v == units - 1, _W_LAG, slot)
                copies.append(
                    pltpu.make_async_copy(
                        buf.at[(pl.ds(s, width), j) + pieces[p]],
                        o_hbm.at[(pl.ds(first + s, width), j) + pieces[p]],
                        w_sem.at[slot],
                    )
                )
            return copies

        def w_wait_unit(narrow, v):
            def wait(width):
                src = buf.at[pl.ds(group_start(narrow, v), width), _mod(v, _Q)]
                pltpu.make_async_copy(src, src, w_sem.at[_mod(v, _W_LAG)]).wait()

            by_width(narrow, v, wait)

        def w_wait_last(c, lo, hi):
            first, _, narrow, units = lookup(c)

            def wait(width):
                for copy in w_copies(first, narrow, units, units - 1, width, lo, hi):
                    copy.wait()

            by_width(narrow, units - 1, wait)

        def normalise(first, s0, count, j):
            means = []
            for i in range(count):
                acc = None
                for rr, cc in tiles:
                    val = buf[s0 + i, j, rr, cc].astype(jnp.float32)
                    acc = val if acc is None else acc + val
                means.append(total(acc) * inv_n)
            affine = []
            for i in range(count):
                acc = None
                for rr, cc in tiles:
                    val = buf[s0 + i, j, rr, cc].astype(jnp.float32) - means[i]
                    val = val * val
                    acc = val if acc is None else acc + val
                ch = _mod((first + s0 + i) * _Q + j, C)
                scale = lax.rsqrt(total(acc) * inv_n + _EPS) * gt[pl.ds(ch, 1), :]
                reps = _C_COLS // _LANES
                affine.append(
                    (
                        jnp.concatenate([scale] * reps, axis=1),
                        jnp.concatenate([bt[pl.ds(ch, 1), :]] * reps, axis=1),
                    )
                )
            for i in range(count):
                scale, shift = affine[i]
                for rr, cc in tiles:
                    val = buf[s0 + i, j, rr, cc].astype(jnp.float32) - means[i]
                    buf[s0 + i, j, rr, cc] = (val * scale + shift).astype(buf.dtype)

        gb_copies = [
            pltpu.make_async_copy(src, gb.at[i], gb_sem)
            for i, src in enumerate((g_hbm, b_hbm))
        ]

        def chunk(c):
            first, columns, narrow, units = lookup(c)

            def read(u):
                pl.when(u >= _R_LAG)(lambda: r_wait_column(u - _R_LAG))
                for i, copy in enumerate(r_copies(first, columns, u, 0, n_pieces)):
                    copy.start(priority=i % 2)

                @pl.when(u == 0)
                def _():
                    @pl.when(c == 0)
                    def _():
                        for copy in gb_copies:
                            copy.start()

                    @pl.when(c > 0)
                    def _():
                        w_wait_last(c - 1, n_pieces - _W_TAIL, n_pieces)

            _loop(0, columns, read)

            @pl.when(c == 0)
            def _():
                for copy in gb_copies:
                    copy.wait()
                for i, dst in enumerate((gt, bt)):
                    val = gb[i].astype(jnp.float32)
                    for t in range(C // _LANES):
                        dst[pl.ds(t * _LANES, _LANES), :] = jnp.broadcast_to(
                            val[t : t + 1, :], (_LANES, _LANES)
                        ).T

            def write(v):
                last = columns - 1

                @pl.when(v == 0)
                def _():
                    for back in range(_R_LAG - 1, 0, -1):
                        r_wait_column(last - back)
                    for copy in r_copies(first, columns, last, 0, n_pieces - _R_TAIL):
                        copy.wait()

                pl.when(v >= _W_LAG)(lambda: w_wait_unit(narrow, v - _W_LAG))

                @pl.when(v >= 0)
                def _():
                    def start(width):
                        for copy in w_copies(first, narrow, units, v, width, 0, n_pieces):
                            copy.start()

                    by_width(narrow, v, start)

                @pl.when(v == 1)
                def _():
                    lo = n_pieces - _R_TAIL
                    for copy in r_copies(first, columns, last, lo, n_pieces):
                        copy.wait()

                @pl.when(v + _AHEAD < units)
                def _():
                    s0, j = group_start(narrow, v + _AHEAD), _mod(v + _AHEAD, _Q)
                    normalise(first, s0, _W_NARROW, j)

                    @pl.when(v + _AHEAD >= narrow)
                    def _():
                        normalise(first, s0 + _W_NARROW, _W_WIDE - _W_NARROW, j)

            _loop(-_AHEAD, units, write)
            for back in range(_W_LAG - 1, 0, -1):
                w_wait_unit(narrow, units - 1 - back)
            w_wait_last(c, 0, n_pieces - _W_TAIL)

        _loop(0, len(plan), chunk)
        w_wait_last(jnp.int32(len(plan) - 1), n_pieces - _W_TAIL, n_pieces)

    scratch = [
        pltpu.VMEM((_CHUNK, _Q, W, H), jnp.bfloat16),
        pltpu.VMEM((2, C // _LANES, _LANES), jnp.bfloat16),
        pltpu.VMEM((C, _LANES), jnp.float32),
        pltpu.VMEM((C, _LANES), jnp.float32),
        pltpu.SemaphoreType.DMA((_R_LAG + 1,)),
        pltpu.SemaphoreType.DMA((_W_LAG + 1,)),
        pltpu.SemaphoreType.DMA,
    ]
    return kernel, scratch


@jax.jit
def pallas_standalone__instancenorm__prompt_kernel(
    x: jax.Array,
    g: jax.Array,
    b: jax.Array,
):
    B, C, H, W = x.shape
    kernel, scratch = _make_kernel(B, C, H, W)
    xt = jnp.transpose(x, (0, 1, 3, 2)).reshape(B * C // _Q, _Q, W, H)
    y = pl.pallas_call(
        kernel,
        in_specs=[pl.BlockSpec(memory_space=pl.ANY)] * 3,
        out_specs=pl.BlockSpec(memory_space=pl.ANY),
        out_shape=jax.ShapeDtypeStruct(xt.shape, xt.dtype),
        scratch_shapes=scratch,
        compiler_params=pltpu.CompilerParams(
            vmem_limit_bytes=120 * 1024 * 1024, disable_bounds_checks=True
        ),
    )(xt, g.reshape(C // _LANES, _LANES), b.reshape(C // _LANES, _LANES))
    return jnp.transpose(y.reshape(B, C, W, H), (0, 1, 3, 2))
```
